```python
import os as _os
_os.environ.setdefault("JAX_PLATFORMS", "cpu")
import jax
import jax.numpy as jnp

def _softmax(x, axis=-1):
    return jax.nn.softmax(x, axis=axis)
def _gelu(x):
    return jax.nn.gelu(x, approximate=True)
def _silu(x):
    return jax.nn.silu(x)
def _sigmoid(x):
    return jax.nn.sigmoid(x)
def _layernorm(x, axis=-1, eps=1e-5):
    m = jnp.mean(x, axis=axis, keepdims=True)
    v = jnp.var(x, axis=axis, keepdims=True)
    return (x - m) / jnp.sqrt(v + eps)
def _scatter_add(tgt, idx, src, axis=0):
    return tgt.at[idx].add(src)
def _segment_sum(src, seg, n):
    return jax.ops.segment_sum(src, seg, n)
class _Rng:
    def __init__(self, key):
        self._k = key
    def _next(self):
        self._k, sub = jax.random.split(self._k)
        return sub
    def normal(self, shape):
        return jax.random.normal(self._next(), shape, dtype=jnp.bfloat16)
    def randint(self, lo, hi, shape):
        return jax.random.randint(self._next(), shape, lo, hi, dtype=jnp.int32)
    def uniform(self, shape, lo=0.0, hi=1.0):
        return jax.random.uniform(self._next(), shape, jnp.bfloat16, lo, hi)
    def permutation(self, n):
        return jax.random.permutation(self._next(), n)


kernel_name = 'sequential_preLN__sliding_local_dilated__dense_activation_mish__prompt'

def setup_inputs():
    _rng = _Rng(jax.random.key(int.from_bytes(__import__("os").urandom(4), "little")))
    _w = (lambda a: (lambda t: t.astype(jnp.bfloat16) if jnp.issubdtype(t.dtype, jnp.floating) else t)(jnp.asarray(a)))
    def _A_setup():
        B, S, D = 1, 2048, 512
        return {
            "x": _w((lambda *s: _rng.normal(s) * 0.05)(B, S, D)),
            "wqkv": _w((lambda *s: _rng.normal(s) * 0.05)(D, 3 * D)),
            "wo": _w((lambda *s: _rng.normal(s) * 0.05)(D, D)),
        }
    _A_in = _A_setup()

    def _B_setup():
        B, S, D, F = 1, 2048, 512, 1376
        return {
            "x": _w((lambda *s: _rng.normal(s) * 0.05)(B, S, D)),
            "w1": _w((lambda *s: _rng.normal(s) * 1.6)(D, F) * (D ** -0.5)),
            "b1": _w((lambda *s: _rng.normal(s) * 0.1)(F)),
            "w2": _w((lambda *s: _rng.normal(s) * 0.1)(F, D) * (F ** -0.5)),
        }
    _B_in = _B_setup()

    return {
        "A_x": _A_in["x"],
        "A_wqkv": _A_in["wqkv"],
        "A_wo": _A_in["wo"],
        "B_x": _B_in["x"],
        "B_w1": _B_in["w1"],
        "B_b1": _B_in["b1"],
        "B_w2": _B_in["w2"],
    }

def reference(A_x, A_wqkv, A_wo, B_x, B_w1, B_b1, B_w2):
    def _A_ref(x, wqkv, wo):
        B, S, D = x.shape
        H = 32; Dh = D // H
        W, dil = 8, 2
        qkv = (lambda x, *d: x.transpose(*d))((x @ wqkv).reshape(B, S, 3, H, Dh), 2, 0, 3, 1, 4)
        q, k, v = qkv[0], qkv[1], qkv[2]
        scale = Dh ** -0.5
        pos = jnp.arange(S)
        off = jnp.arange(W) * dil
        idx = pos[:, None] - off[None, :]
        mask = idx >= 0
        idx_c = jnp.where(mask, idx, 0).reshape(-1)
        kg = k[:, :, idx_c, :].reshape(B, H, S, W, Dh)
        vg = v[:, :, idx_c, :].reshape(B, H, S, W, Dh)
        logits = jnp.einsum("bhsd,bhswd->bhsw", q, kg) * scale
        logits = jnp.where(mask[None, None, :, :], logits, -1e9)
        attn = _softmax(logits, axis=-1)
        o = jnp.einsum("bhsw,bhswd->bhsd", attn, vg)
        return (lambda x, *d: x.transpose(*d))(o, 0, 2, 1, 3).reshape(B, S, D) @ wo

    def _B_ref(x, w1, b1, w2):
        h = jnp.einsum("bsd,df->bsf", x, w1) + b1
        sp = jnp.log1p(jnp.exp(-jnp.abs(h))) + jnp.where(h > 0, h, jnp.zeros_like(h))
        act = h * jnp.tanh(sp)
        return jnp.einsum("bsf,fd->bsd", act, w2)

    x = A_x
    h = x + _A_ref(_layernorm(x, axis=-1), A_wqkv, A_wo)
    h2 = h + _B_ref(_layernorm(h, axis=-1), B_w1, B_b1, B_w2)
    return h2
```

```python
import functools

import jax
import jax.numpy as jnp
import jax.experimental.pallas as pl
import jax.experimental.pallas.tpu as pltpu

_H = 32
_DH = 16
_W = 8
_DIL = 2
_HALO = 16
_EPS = 1e-5


def _layernorm(x):
    m = jnp.mean(x, axis=-1, keepdims=True)
    xc = x - m
    v = jnp.mean(xc * xc, axis=-1, keepdims=True)
    return xc * jax.lax.rsqrt(v + _EPS)


def _mish(h):
    n = jnp.exp(-jnp.abs(h))
    n2 = n * n
    pos = h > 0
    num = jnp.where(pos, 1.0 + 2.0 * n, n2 + 2.0 * n)
    den = jnp.where(pos, 1.0 + 2.0 * n + 2.0 * n2, n2 + 2.0 * n + 2.0)
    return h * (num / den)


def _kernel(x_ref, wqkv_ref, wo_ref, w1_ref, b1_ref, w2_ref, o_ref, kv_scr):
    i = pl.program_id(0)
    T, D = x_ref.shape
    f32 = jnp.float32
    bf16 = jnp.bfloat16

    x = x_ref[...].astype(f32)
    ln1 = _layernorm(x).astype(bf16)
    qkv = jnp.dot(ln1, wqkv_ref[...], preferred_element_type=f32)

    @pl.when(i == 0)
    def _():
        kv_scr[0:_HALO, :] = jnp.zeros((_HALO, 2 * D), f32)

    @pl.when(i > 0)
    def _():
        kv_scr[0:_HALO, :] = kv_scr[T:T + _HALO, :]

    kv_scr[_HALO:_HALO + T, :] = qkv[:, D:]
    q = qkv[:, :D] * (_DH ** -0.5)

    pos = i * T + jax.lax.broadcasted_iota(jnp.int32, (T, 128), 0)
    logits = []
    for w in range(_W):
        kw = kv_scr[pl.ds(_HALO - _DIL * w, T), 0:D]
        prod = q * kw
        part = prod[:, 0:128]
        for c in range(1, D // 128):
            part = part + prod[:, c * 128:(c + 1) * 128]
        part = part + pltpu.roll(part, 32, 1)
        part = part + pltpu.roll(part, 64, 1)
        if w > 0:
            part = jnp.where(pos >= _DIL * w, part, -1e9)
        logits.append(part)
    m = logits[0]
    for w in range(1, _W):
        m = jnp.maximum(m, logits[w])
    es = [jnp.exp(l - m) for l in logits]
    s = es[0]
    for w in range(1, _W):
        s = s + es[w]
    inv = 1.0 / s
    cols = []
    for c in range(D // 128):
        acc = None
        for w in range(_W):
            vw = kv_scr[pl.ds(_HALO - _DIL * w, T), D + c * 128:D + (c + 1) * 128]
            t = es[w] * vw
            acc = t if acc is None else acc + t
        cols.append(acc * inv)
    o = jnp.concatenate(cols, axis=1).astype(bf16)
    h = x + jnp.dot(o, wo_ref[...], preferred_element_type=f32)

    ln2 = _layernorm(h).astype(bf16)
    h1 = jnp.dot(ln2, w1_ref[...], preferred_element_type=f32) + b1_ref[...].astype(f32)
    act = _mish(h1).astype(bf16)
    out = h + jnp.dot(act, w2_ref[...], preferred_element_type=f32)
    o_ref[...] = out.astype(o_ref.dtype)


@jax.jit
def pallas_sequential_preLN__sliding_local_dilated__dense_activation_mish__prompt_kernel(
    A_x: jax.Array,
    A_wqkv: jax.Array,
    A_wo: jax.Array,
    B_x: jax.Array,
    B_w1: jax.Array,
    B_b1: jax.Array,
    B_w2: jax.Array,
):
    B, S, D = A_x.shape
    F = B_w1.shape[1]
    T = 256
    x2 = A_x.reshape(B * S, D)
    wqkv_p = A_wqkv.reshape(D, 3, _H, _DH).transpose(0, 1, 3, 2).reshape(D, 3 * D)
    wo_p = A_wo.reshape(_H, _DH, D).transpose(1, 0, 2).reshape(D, D)
    b1 = B_b1.reshape(1, F)

    out = pl.pallas_call(
        _kernel,
        grid=(S // T,),
        in_specs=[
            pl.BlockSpec((T, D), lambda i: (i, 0)),
            pl.BlockSpec((D, 3 * D), lambda i: (0, 0)),
            pl.BlockSpec((D, D), lambda i: (0, 0)),
            pl.BlockSpec((D, F), lambda i: (0, 0)),
            pl.BlockSpec((1, F), lambda i: (0, 0)),
            pl.BlockSpec((F, D), lambda i: (0, 0)),
        ],
        out_specs=pl.BlockSpec((T, D), lambda i: (i, 0)),
        out_shape=jax.ShapeDtypeStruct((B * S, D), A_x.dtype),
        scratch_shapes=[pltpu.VMEM((T + _HALO, 2 * D), jnp.float32)],
        compiler_params=pltpu.CompilerParams(
            dimension_semantics=("arbitrary",),
            vmem_limit_bytes=64 * 1024 * 1024,
        ),
    )(x2, wqkv_p, wo_p, B_w1, b1, B_w2)
    return out.reshape(B, S, D)
```

```python
import functools

import jax
import jax.numpy as jnp
import jax.experimental.pallas as pl
import jax.experimental.pallas.tpu as pltpu

_H = 32
_DH = 16
_W = 8
_DIL = 2
_HALO = 16
_EPS = 1e-5
_T = 512
_SUB = 128


def _layernorm(x):
    m = jnp.mean(x, axis=-1, keepdims=True)
    xc = x - m
    v = jnp.mean(xc * xc, axis=-1, keepdims=True)
    return xc * jax.lax.rsqrt(v + _EPS)


def _mish(h):
    e = jnp.exp(jnp.minimum(h, 20.0))
    t = e * (e + 2.0)
    return h * (t / (t + 2.0))


def _kernel(x_ref, wqkv_hbm, wo_hbm, w1_hbm, b1_ref, w2_hbm, o_ref,
            kv_scr, wqkv_raw, wqkv_p, wo_raw, wo_p, w1_v, w2_v, sems):
    i = pl.program_id(0)
    T, D = x_ref.shape
    f32 = jnp.float32
    bf16 = jnp.bfloat16
    nsub = T // _SUB

    def wqkv_copy(j):
        return pltpu.make_async_copy(wqkv_hbm.at[:, j * D:(j + 1) * D],
                                     wqkv_raw.at[:, j * D:(j + 1) * D], sems.at[3 + j])

    def w1_copy():
        return pltpu.make_async_copy(w1_hbm, w1_v, sems.at[0])

    def w2_copy():
        return pltpu.make_async_copy(w2_hbm, w2_v, sems.at[1])

    def wo_copy():
        return pltpu.make_async_copy(wo_hbm, wo_raw, sems.at[2])

    @pl.when(i == 0)
    def _():
        for j in range(3):
            wqkv_copy(j).start()
        wo_copy().start()
        w1_copy().start()
        w2_copy().start()
        kv_scr[0:_HALO, :] = jnp.zeros((_HALO, 2 * D), f32)
        src = jax.lax.broadcasted_iota(jnp.int32, (D, D), 0)
        dst = jax.lax.broadcasted_iota(jnp.int32, (D, D), 1)
        perm = jnp.where((dst % _H) * _DH + dst // _H == src, 1.0, 0.0).astype(bf16)
        for j in range(3):
            wqkv_copy(j).wait()
            wqkv_p[:, j * D:(j + 1) * D] = jnp.dot(
                wqkv_raw[:, j * D:(j + 1) * D], perm,
                preferred_element_type=f32).astype(bf16)
        perm_t = jnp.where((src % _H) * _DH + src // _H == dst, 1.0, 0.0).astype(bf16)
        wo_copy().wait()
        wo_p[...] = jnp.dot(perm_t, wo_raw[...], preferred_element_type=f32).astype(bf16)
        w1_copy().wait()
        w2_copy().wait()

    @pl.when(i > 0)
    def _():
        kv_scr[0:_HALO, :] = kv_scr[T:T + _HALO, :]

    def stage_qkv(sb):
        r0 = sb * _SUB
        x = x_ref[r0:r0 + _SUB, :].astype(f32)
        ln1 = _layernorm(x).astype(bf16)
        qkv = jnp.dot(ln1, wqkv_p[...], preferred_element_type=f32)
        kv_scr[_HALO + r0:_HALO + r0 + _SUB, :] = qkv[:, D:]
        return qkv[:, :D] * (_DH ** -0.5)

    def stage_attn(sb, q):
        r0 = sb * _SUB
        pos = i * T + r0 + jax.lax.broadcasted_iota(jnp.int32, (_SUB, 128), 0)
        logits = []
        for w in range(_W):
            kw = kv_scr[pl.ds(_HALO + r0 - _DIL * w, _SUB), 0:D]
            prod = q * kw
            part = prod[:, 0:128]
            for c in range(1, D // 128):
                part = part + prod[:, c * 128:(c + 1) * 128]
            part = part + pltpu.roll(part, 32, 1)
            part = part + pltpu.roll(part, 64, 1)
            if w > 0:
                part = jnp.where(pos >= _DIL * w, part, -1e9)
            logits.append(part)
        m = logits[0]
        for w in range(1, _W):
            m = jnp.maximum(m, logits[w])
        es = [jnp.exp(l - m) for l in logits]
        s = es[0]
        for w in range(1, _W):
            s = s + es[w]
        inv = 1.0 / s
        cols = []
        for c in range(D // 128):
            acc = None
            for w in range(_W):
                vw = kv_scr[pl.ds(_HALO + r0 - _DIL * w, _SUB), D + c * 128:D + (c + 1) * 128]
                t = es[w] * vw
                acc = t if acc is None else acc + t
            cols.append(acc * inv)
        return jnp.concatenate(cols, axis=1).astype(bf16)

    def stage_wo(sb, o):
        r0 = sb * _SUB
        x = x_ref[r0:r0 + _SUB, :].astype(f32)
        h = x + jnp.dot(o, wo_p[...], preferred_element_type=f32)
        return h, _layernorm(h).astype(bf16)

    def stage_ffn(sb, h, ln2):
        r0 = sb * _SUB
        h1 = jax.lax.dot_general(ln2, w1_v[...], (((1,), (1,)), ((), ())),
                                 preferred_element_type=f32) + b1_ref[...].astype(f32)
        act = _mish(h1).astype(bf16)
        out = h + jnp.dot(act, w2_v[...], preferred_element_type=f32)
        o_ref[r0:r0 + _SUB, :] = out.astype(o_ref.dtype)

    qs = [stage_qkv(sb) for sb in range(nsub)]
    os_ = [stage_attn(sb, qs[sb]) for sb in range(nsub)]
    hs = [stage_wo(sb, os_[sb]) for sb in range(nsub)]
    for sb in range(nsub):
        stage_ffn(sb, *hs[sb])


@jax.jit
def pallas_sequential_preLN__sliding_local_dilated__dense_activation_mish__prompt_kernel(
    A_x: jax.Array,
    A_wqkv: jax.Array,
    A_wo: jax.Array,
    B_x: jax.Array,
    B_w1: jax.Array,
    B_b1: jax.Array,
    B_w2: jax.Array,
):
    B, S, D = A_x.shape
    F = B_w1.shape[1]
    T = _T
    x2 = A_x.reshape(B * S, D)
    b1 = B_b1.reshape(1, F)
    bf16 = jnp.bfloat16

    out = pl.pallas_call(
        _kernel,
        grid=(S // T,),
        in_specs=[
            pl.BlockSpec((T, D), lambda i: (i, 0)),
            pl.BlockSpec(memory_space=pl.ANY),
            pl.BlockSpec(memory_space=pl.ANY),
            pl.BlockSpec(memory_space=pl.ANY),
            pl.BlockSpec((1, F), lambda i: (0, 0)),
            pl.BlockSpec(memory_space=pl.ANY),
        ],
        out_specs=pl.BlockSpec((T, D), lambda i: (i, 0)),
        out_shape=jax.ShapeDtypeStruct((B * S, D), A_x.dtype),
        scratch_shapes=[
            pltpu.VMEM((T + _HALO, 2 * D), jnp.float32),
            pltpu.VMEM((D, 3 * D), bf16),
            pltpu.VMEM((D, 3 * D), bf16),
            pltpu.VMEM((D, D), bf16),
            pltpu.VMEM((D, D), bf16),
            pltpu.VMEM((F, D), bf16),
            pltpu.VMEM((F, D), bf16),
            pltpu.SemaphoreType.DMA((6,)),
        ],
        compiler_params=pltpu.CompilerParams(
            dimension_semantics=("arbitrary",),
            vmem_limit_bytes=64 * 1024 * 1024,
        ),
    )(x2, A_wqkv, A_wo, B_w1.T, b1, B_w2)
    return out.reshape(B, S, D)
```
